```python
import os as _os
_os.environ.setdefault("JAX_PLATFORMS", "cpu")
import jax
import jax.numpy as jnp

def _softmax(x, axis=-1):
    return jax.nn.softmax(x, axis=axis)
def _gelu(x):
    return jax.nn.gelu(x, approximate=True)
def _silu(x):
    return jax.nn.silu(x)
def _sigmoid(x):
    return jax.nn.sigmoid(x)
def _layernorm(x, axis=-1, eps=1e-5):
    m = jnp.mean(x, axis=axis, keepdims=True)
    v = jnp.var(x, axis=axis, keepdims=True)
    return (x - m) / jnp.sqrt(v + eps)
def _scatter_add(tgt, idx, src, axis=0):
    return tgt.at[idx].add(src)
def _segment_sum(src, seg, n):
    return jax.ops.segment_sum(src, seg, n)
class _Rng:
    def __init__(self, key):
        self._k = key
    def _next(self):
        self._k, sub = jax.random.split(self._k)
        return sub
    def normal(self, shape):
        return jax.random.normal(self._next(), shape, dtype=jnp.bfloat16)
    def randint(self, lo, hi, shape):
        return jax.random.randint(self._next(), shape, lo, hi, dtype=jnp.int32)
    def uniform(self, shape, lo=0.0, hi=1.0):
        return jax.random.uniform(self._next(), shape, jnp.bfloat16, lo, hi)
    def permutation(self, n):
        return jax.random.permutation(self._next(), n)


kernel_name = 'standalone__mha_softmax__near_ridge'

def setup_inputs():
    _rng = _Rng(jax.random.key(int.from_bytes(__import__("os").urandom(4), "little")))
    _w = (lambda a: (lambda t: t.astype(jnp.bfloat16) if jnp.issubdtype(t.dtype, jnp.floating) else t)(jnp.asarray(a)))
    B, H, Sq, Sk, D = 8, 32, 304, 2048, 128
    return {
        "q": _w((lambda *s: _rng.normal(s) * 0.4)(B, H, Sq, D)),
        "k": _w((lambda *s: _rng.normal(s) * 0.4)(B, H, Sk, D)),
        "v": _w((lambda *s: _rng.normal(s) * 0.05)(B, H, Sk, D)),
    }

def reference(q, k, v):
    scale = q.shape[-1] ** -0.5
    scores = jnp.einsum("bhqd,bhkd->bhqk", q, k) * scale
    p = _softmax(scores, axis=-1)
    return jnp.einsum("bhqk,bhkd->bhqd", p, v)
```

```python
import math

import jax
import jax.numpy as jnp
import jax.experimental.pallas as pl
import jax.experimental.pallas.tpu as pltpu


def _kernel(q_ref, k_ref, v_ref, o_ref):
    q = q_ref[0]
    k = k_ref[0]
    v = v_ref[0]
    d = q.shape[-1]
    c = (d ** -0.5) * math.log2(math.e)
    s = jax.lax.dot_general(q, k, (((1,), (1,)), ((), ())),
                            preferred_element_type=jnp.float32)
    m = jnp.max(s, axis=-1, keepdims=True)
    p = jnp.exp2((s - m) * c)
    l = jnp.sum(p, axis=-1, keepdims=True)
    o = jnp.dot(p.astype(v.dtype), v, preferred_element_type=jnp.float32)
    o_ref[0] = (o / l).astype(o_ref.dtype)


@jax.jit
def pallas_standalone__mha_softmax__near_ridge_kernel(
    q: jax.Array,
    k: jax.Array,
    v: jax.Array,
):
    B, H, Sq, D = q.shape
    Sk = k.shape[2]
    q3 = q.reshape(B * H, Sq, D)
    k3 = k.reshape(B * H, Sk, D)
    v3 = v.reshape(B * H, Sk, D)
    out = pl.pallas_call(
        _kernel,
        grid=(B * H,),
        in_specs=[
            pl.BlockSpec((1, Sq, D), lambda i: (i, 0, 0)),
            pl.BlockSpec((1, Sk, D), lambda i: (i, 0, 0)),
            pl.BlockSpec((1, Sk, D), lambda i: (i, 0, 0)),
        ],
        out_specs=pl.BlockSpec((1, Sq, D), lambda i: (i, 0, 0)),
        out_shape=jax.ShapeDtypeStruct((B * H, Sq, D), q.dtype),
        compiler_params=pltpu.CompilerParams(
            dimension_semantics=("parallel",),
            vmem_limit_bytes=64 * 1024 * 1024,
        ),
    )(q3, k3, v3)
    return out.reshape(B, H, Sq, D)
```

```python
import math
import jax
import jax.numpy as jnp
import jax.experimental.pallas as pl
import jax.experimental.pallas.tpu as pltpu

U = 16
FLAGS = {'XLA_TPU_RESCHEDULE_DMA_DONES': True}
DBC = True
RCP = 2
QH = 1
OH = 1
KAHEAD = 0

def _rcp(l):
    if RCP == 0:
        return 1.0 / l
    r = pl.reciprocal(l, approx=True)
    for _ in range(RCP - 1):
        r = r * (2.0 - l * r)
    return r

def _kernel(q_hbm, k_hbm, v_hbm, o_hbm, qb, kb, vb, ob, sq, sk, sv, so):
    NH, Sq, D = q_hbm.shape
    NI = NH // U
    c = (D ** -0.5) * math.log2(math.e)

    def ck(h, g): return pltpu.make_async_copy(k_hbm.at[h], kb.at[g], sk.at[g])
    def cv(h, g): return pltpu.make_async_copy(v_hbm.at[h], vb.at[g], sv.at[g])
    def cqh(h, g): return pltpu.make_async_copy(q_hbm.at[h], qb.at[0, g], sq.at[g])
    def cqb(it, par): return pltpu.make_async_copy(q_hbm.at[pl.ds(it * U, U)], qb.at[par], sq.at[par])
    def coh(h, g): return pltpu.make_async_copy(ob.at[0, g], o_hbm.at[h], so.at[g])
    def cob(it, par): return pltpu.make_async_copy(ob.at[par], o_hbm.at[pl.ds(it * U, U)], so.at[par])

    if not QH:
        cqb(0, 0).start()
    def pro(g, _):
        if QH:
            cqh(g, g).start()
        ck(g, g).start()
        cv(g, g).start()
        return 0
    jax.lax.fori_loop(0, U, pro, 0)

    def body(i, par):
        npar = 1 - par
        more = i + 1 < NI
        if not OH:
            @pl.when(i > 0)
            def _():
                cob(i - 1, npar).start()
            @pl.when(i > 1)
            def _():
                cob(i - 2, par).wait()
        if not QH:
            cqb(i, par).wait()
            @pl.when(more)
            def _():
                cqb(i + 1, npar).start()
        if KAHEAD:
            ck(i * U, 0).wait()
        outs = []
        for g in range(U):
            h = i * U + g
            if QH:
                cqh(h, g).wait()
            if not KAHEAD:
                ck(h, g).wait()
            q = qb[0 if QH else par, g]; k = kb[g]
            s = jax.lax.dot_general(q, k, (((1,), (1,)), ((), ())), preferred_element_type=jnp.float32)
            @pl.when(more)
            def _():
                ck(h + U, g).start()
            if QH:
                @pl.when(more)
                def _():
                    cqh(h + U, g).start()
            m = jnp.max(s, axis=-1, keepdims=True)
            cv(h, g).wait()
            if KAHEAD and g + 1 < U:
                ck(h + 1, g + 1).wait()
            p = jnp.exp2((s - m) * c)
            l = jnp.sum(p, axis=-1, keepdims=True)
            v = vb[g]
            o = jnp.dot(p.astype(v.dtype), v, preferred_element_type=jnp.float32)
            @pl.when(more)
            def _():
                cv(h + U, g).start()
            out = (o * _rcp(l)).astype(ob.dtype)
            if OH:
                @pl.when(i > 0)
                def _():
                    coh(h - U, g).wait()
                ob[0, g] = out
                coh(h, g).start()
            else:
                outs.append(out)
        if not OH:
            for g in range(U):
                ob[par, g] = outs[g]
        return npar

    jax.lax.fori_loop(0, NI, body, jnp.int32(0))
    if OH:
        for g in range(U):
            coh((NI - 1) * U + g, g).wait()
    else:
        cob(NI - 2, (NI - 2) % 2).wait()
        cob(NI - 1, (NI - 1) % 2).start()
        cob(NI - 1, (NI - 1) % 2).wait()

@jax.jit
def pallas_standalone__mha_softmax__near_ridge_kernel(q, k, v):
    B, H, Sq, D = q.shape
    Sk = k.shape[2]
    q3 = q.reshape(B * H, Sq, D)
    k3 = k.reshape(B * H, Sk, D)
    v3 = v.reshape(B * H, Sk, D)
    out = pl.pallas_call(
        _kernel,
        in_specs=[pl.BlockSpec(memory_space=pl.ANY)] * 3,
        out_specs=pl.BlockSpec(memory_space=pl.ANY),
        out_shape=jax.ShapeDtypeStruct((B * H, Sq, D), q.dtype),
        scratch_shapes=[
            pltpu.VMEM((1 if QH else 2, U, Sq, D), q.dtype), pltpu.VMEM((U, Sk, D), q.dtype),
            pltpu.VMEM((U, Sk, D), q.dtype), pltpu.VMEM((1 if OH else 2, U, Sq, D), q.dtype),
            pltpu.SemaphoreType.DMA((U if QH else 2,)), pltpu.SemaphoreType.DMA((U,)),
            pltpu.SemaphoreType.DMA((U,)), pltpu.SemaphoreType.DMA((U if OH else 2,)),
        ],
        compiler_params=pltpu.CompilerParams(vmem_limit_bytes=120 * 1024 * 1024, flags=FLAGS,
                                             disable_bounds_checks=DBC),
    )(q3, k3, v3)
    return out.reshape(B, H, Sq, D)
```

```python
import math
import jax
import jax.numpy as jnp
import jax.experimental.pallas as pl
import jax.experimental.pallas.tpu as pltpu

U = 16
OG = 2
FLAGS = {'XLA_TPU_RESCHEDULE_DMA_DONES': True}
DBC = True
RCP = 2
TIED = 2
TIEC = 1
PIN = 0
POUT = 0

def _rcp(l):
    if RCP == 0:
        return 1.0 / l
    r = pl.reciprocal(l, approx=True)
    for _ in range(RCP - 1):
        r = r * (2.0 - l * r)
    return r

def _partial(p):
    n = p.shape[1] // 128
    lp = p[:, :128]
    for j in range(1, n):
        lp = lp + p[:, j * 128:(j + 1) * 128]
    return lp

def _finish(o, lp):
    return o * _rcp(jnp.sum(lp, axis=-1, keepdims=True))

def _kernel(q_hbm, k_hbm, v_hbm, o_hbm, qb, kb, vb, acc_c, lp_c, zs, sq, sk, sv, so):
    NH, Sq, D = q_hbm.shape
    Sk = k_hbm.shape[1]
    NI = NH // U
    NG = U // OG
    c = (D ** -0.5) * math.log2(math.e)

    def ck(h, g): return pltpu.make_async_copy(k_hbm.at[h], kb.at[g, pl.ds(0, Sk)], sk.at[g])
    def cv(h, g): return pltpu.make_async_copy(v_hbm.at[h], vb.at[g], sv.at[g])
    def cq(h, g): return pltpu.make_async_copy(q_hbm.at[h], qb.at[g], sq.at[g])
    def co(it, j):
        return pltpu.make_async_copy(kb.at[pl.ds(j * OG, OG), pl.ds(Sk, Sq)],
                                     o_hbm.at[pl.ds(it * U + j * OG, OG)], so.at[j])

    def pro(g, _):
        cq(g, g).start(priority=PIN)
        ck(g, g).start(priority=PIN)
        cv(g, g).start(priority=PIN)
        return 0
    jax.lax.fori_loop(0, U, pro, 0)
    zs[0] = 0
    acc_c[...] = jnp.zeros(acc_c.shape, acc_c.dtype)
    lp_c[...] = jnp.ones(lp_c.shape, lp_c.dtype)

    def carried():
        return _finish(acc_c[...], lp_c[...]).astype(kb.dtype)

    def body(i, _):
        more = i + 1 < NI
        zo = zs[0]
        def emit(it, g, out, carried_head):
            if g % OG == 0:
                @pl.when(it > 0)
                def _():
                    co(it - 1, g // OG).wait()
            kb[g + zo, pl.ds(Sk, Sq), :] = out
            if g % OG == OG - 1:
                if carried_head:
                    @pl.when(it >= 0)
                    def _():
                        co(it, g // OG).start(priority=POUT)
                else:
                    co(it, g // OG).start(priority=POUT)
        pend = [(TIEC, (i - 1, U - 1, carried(), True))]
        for g in range(U):
            h = i * U + g
            while pend and pend[0][0] <= g:
                emit(*pend.pop(0)[1])
            cq(h, g).wait()
            ck(h, g).wait()
            s = jax.lax.dot_general(qb[g], kb[g, :Sk], (((1,), (1,)), ((), ())), preferred_element_type=jnp.float32)
            @pl.when(more)
            def _():
                ck(h + U, g).start(priority=PIN)
            @pl.when(more)
            def _():
                cq(h + U, g).start(priority=PIN)
            m = jnp.max(s, axis=-1, keepdims=True)
            cv(h, g).wait()
            p = jnp.exp2((s - m) * c)
            o = jnp.dot(p.astype(vb.dtype), vb[g], preferred_element_type=jnp.float32)
            @pl.when(more)
            def _():
                cv(h + U, g).start(priority=PIN)
            if g == U - 1:
                cval = (o, _partial(p))
            else:
                pend.append((g + TIED, (i, g, _finish(o, _partial(p)).astype(kb.dtype), False)))
        while pend:
            emit(*pend.pop(0)[1])
        acc_c[...] = cval[0]
        lp_c[...] = cval[1]
        return 0

    jax.lax.fori_loop(0, NI, body, 0)
    if OG == 1:
        co(NI - 2, U - 1).wait()
    kb[U - 1, pl.ds(Sk, Sq), :] = carried()
    co(NI - 1, NG - 1).start(priority=POUT)
    for j in range(NG):
        co(NI - 1, j).wait()

@jax.jit
def pallas_standalone__mha_softmax__near_ridge_kernel(q, k, v):
    B, H, Sq, D = q.shape
    Sk = k.shape[2]
    q3 = q.reshape(B * H, Sq, D)
    k3 = k.reshape(B * H, Sk, D)
    v3 = v.reshape(B * H, Sk, D)
    out = pl.pallas_call(
        _kernel,
        in_specs=[pl.BlockSpec(memory_space=pl.ANY)] * 3,
        out_specs=pl.BlockSpec(memory_space=pl.ANY),
        out_shape=jax.ShapeDtypeStruct((B * H, Sq, D), q.dtype),
        scratch_shapes=[
            pltpu.VMEM((U, Sq, D), q.dtype),
            pltpu.VMEM((U, Sk + Sq, D), q.dtype),
            pltpu.VMEM((U, Sk, D), q.dtype),
            pltpu.VMEM((Sq, D), jnp.float32),
            pltpu.VMEM((Sq, 128), jnp.float32),
            pltpu.SMEM((1,), jnp.int32),
            pltpu.SemaphoreType.DMA((U,)), pltpu.SemaphoreType.DMA((U,)),
            pltpu.SemaphoreType.DMA((U,)), pltpu.SemaphoreType.DMA((U // OG,)),
        ],
        compiler_params=pltpu.CompilerParams(vmem_limit_bytes=120 * 1024 * 1024, flags=FLAGS,
                                             disable_bounds_checks=DBC),
    )(q3, k3, v3)
    return out.reshape(B, H, Sq, D)
```

```python
import math

import jax
import jax.numpy as jnp
import jax.experimental.pallas as pl
import jax.experimental.pallas.tpu as pltpu

HEADS_PER_STEP = 16
OUT_GROUP = 8
STORE_LAG = 2
LANES = 128


def _attention_kernel(
    q_hbm, k_hbm, v_hbm, o_hbm,
    kqo_buf, v_buf, acc_carry, sum_carry, zero_smem, kq_sem, v_sem, o_sem,
):
  num_heads, sq, d = q_hbm.shape
  sk = k_hbm.shape[1]
  step = HEADS_PER_STEP
  num_steps = num_heads // step
  num_groups = step // OUT_GROUP
  q_row, o_row = sk, sk + sq
  c = (d ** -0.5) * math.log2(math.e)

  def k_copy(h, slot):
    return pltpu.make_async_copy(
        k_hbm.at[h], kqo_buf.at[slot, pl.ds(0, sk)], kq_sem.at[slot])

  def q_copy(h, slot):
    return pltpu.make_async_copy(
        q_hbm.at[h], kqo_buf.at[slot, pl.ds(q_row, sq)], kq_sem.at[slot])

  def wait_kq(slot):
    both = kqo_buf.at[slot, pl.ds(0, sk + sq)]
    pltpu.make_async_copy(both, both, kq_sem.at[slot]).wait()

  def v_copy(h, slot):
    return pltpu.make_async_copy(v_hbm.at[h], v_buf.at[slot], v_sem.at[slot])

  def o_copy(i, j):
    return pltpu.make_async_copy(
        kqo_buf.at[pl.ds(j * OUT_GROUP, OUT_GROUP), pl.ds(o_row, sq)],
        o_hbm.at[pl.ds(i * step - 1 + j * OUT_GROUP, OUT_GROUP)],
        o_sem.at[j])

  def o_copy_first():
    return pltpu.make_async_copy(
        kqo_buf.at[pl.ds(1, OUT_GROUP - 1), pl.ds(o_row, sq)],
        o_hbm.at[pl.ds(0, OUT_GROUP - 1)],
        o_sem.at[0])

  def o_copy_last():
    return pltpu.make_async_copy(
        kqo_buf.at[0, pl.ds(o_row, sq)], o_hbm.at[num_heads - 1], o_sem.at[0])

  def lane_partial_sums(p):
    part = p[:, :LANES]
    for j in range(1, p.shape[1] // LANES):
      part = part + p[:, j * LANES:(j + 1) * LANES]
    return part

  def normalise(acc, part):
    inv = pltpu.reciprocal(jnp.sum(part, axis=-1, keepdims=True), approx=True)
    return (acc * inv).astype(kqo_buf.dtype)

  def start_first(g, carry):
    k_copy(g, g).start()
    q_copy(g, g).start()
    v_copy(g, g).start()
    return carry

  jax.lax.fori_loop(0, step, start_first, 0)
  zero_smem[0] = 0
  acc_carry[...] = jnp.zeros(acc_carry.shape, acc_carry.dtype)
  sum_carry[...] = jnp.ones(sum_carry.shape, sum_carry.dtype)

  def step_body(i, carry):
    refill = i + 1 < num_steps
    zero = zero_smem[0]

    def stage_output(pos, value):
      group, within = divmod(pos, OUT_GROUP)
      if within == 0:
        if group == 0:
          @pl.when(i == 1)
          def _():
            o_copy_first().wait()

          @pl.when(i > 1)
          def _():
            o_copy(i - 1, 0).wait()
        else:
          @pl.when(i > 0)
          def _():
            o_copy(i - 1, group).wait()

      slot = jnp.clip(pos + zero, 0, step - 1)
      kqo_buf[slot, pl.ds(o_row, sq), :] = value

      if within == OUT_GROUP - 1:
        if group == 0:
          @pl.when(i == 0)
          def _():
            o_copy_first().start()

          @pl.when(i > 0)
          def _():
            o_copy(i, 0).start()
        else:
          o_copy(i, group).start()

    pending = [(STORE_LAG, 0, normalise(acc_carry[...], sum_carry[...]))]

    for g in range(step):
      h = i * step + g
      while pending and pending[0][0] <= g:
        stage_output(*pending.pop(0)[1:])

      wait_kq(g)
      s = jax.lax.dot_general(
          kqo_buf[g, q_row:o_row], kqo_buf[g, :sk],
          (((1,), (1,)), ((), ())), preferred_element_type=jnp.float32)

      @pl.when(refill)
      def _():
        k_copy(h + step, g).start()

      @pl.when(refill)
      def _():
        q_copy(h + step, g).start()

      m = jnp.max(s, axis=-1, keepdims=True)
      v_copy(h, g).wait()
      p = jnp.exp2((s - m) * c)
      acc = jnp.dot(p.astype(v_buf.dtype), v_buf[g],
                    preferred_element_type=jnp.float32)

      @pl.when(refill)
      def _():
        v_copy(h + step, g).start()

      if g + 1 < step:
        pending.append(
            (g + STORE_LAG, g + 1, normalise(acc, lane_partial_sums(p))))
      else:
        last_acc, last_part = acc, lane_partial_sums(p)

    while pending:
      stage_output(*pending.pop(0)[1:])
    acc_carry[...] = last_acc
    sum_carry[...] = last_part
    return carry

  jax.lax.fori_loop(0, num_steps, step_body, 0)

  o_copy(num_steps - 1, 0).wait()
  kqo_buf[0, pl.ds(o_row, sq), :] = normalise(acc_carry[...], sum_carry[...])
  o_copy_last().start()
  for j in range(1, num_groups):
    o_copy(num_steps - 1, j).wait()
  o_copy_last().wait()


@jax.jit
def pallas_standalone__mha_softmax__near_ridge_kernel(
    q: jax.Array,
    k: jax.Array,
    v: jax.Array,
):
  b, h, sq, d = q.shape
  sk = k.shape[2]
  num_heads = b * h
  assert num_heads % HEADS_PER_STEP == 0 and num_heads >= 2 * HEADS_PER_STEP
  assert HEADS_PER_STEP % OUT_GROUP == 0 and OUT_GROUP >= 2
  assert sk % LANES == 0 and d == LANES and sq % 16 == 0

  any_spec = pl.BlockSpec(memory_space=pl.ANY)
  out = pl.pallas_call(
      _attention_kernel,
      in_specs=[any_spec, any_spec, any_spec],
      out_specs=any_spec,
      out_shape=jax.ShapeDtypeStruct((num_heads, sq, d), q.dtype),
      scratch_shapes=[
          pltpu.VMEM((HEADS_PER_STEP, sk + 2 * sq, d), k.dtype),
          pltpu.VMEM((HEADS_PER_STEP, sk, d), v.dtype),
          pltpu.VMEM((sq, d), jnp.float32),
          pltpu.VMEM((sq, LANES), jnp.float32),
          pltpu.SMEM((1,), jnp.int32),
          pltpu.SemaphoreType.DMA((HEADS_PER_STEP,)),
          pltpu.SemaphoreType.DMA((HEADS_PER_STEP,)),
          pltpu.SemaphoreType.DMA((HEADS_PER_STEP // OUT_GROUP,)),
      ],
      compiler_params=pltpu.CompilerParams(
          vmem_limit_bytes=100 * 1024 * 1024,
          disable_bounds_checks=True,
          flags={"XLA_TPU_RESCHEDULE_DMA_DONES": True},
      ),
  )(
      q.reshape(num_heads, sq, d),
      k.reshape(num_heads, sk, d),
      v.reshape(num_heads, sk, d),
  )
  return out.reshape(b, h, sq, d)
```
